```python
import os as _os
_os.environ.setdefault("JAX_PLATFORMS", "cpu")
import jax
import jax.numpy as jnp

def _softmax(x, axis=-1):
    return jax.nn.softmax(x, axis=axis)
def _gelu(x):
    return jax.nn.gelu(x, approximate=True)
def _silu(x):
    return jax.nn.silu(x)
def _sigmoid(x):
    return jax.nn.sigmoid(x)
def _layernorm(x, axis=-1, eps=1e-5):
    m = jnp.mean(x, axis=axis, keepdims=True)
    v = jnp.var(x, axis=axis, keepdims=True)
    return (x - m) / jnp.sqrt(v + eps)
def _scatter_add(tgt, idx, src, axis=0):
    return tgt.at[idx].add(src)
def _segment_sum(src, seg, n):
    return jax.ops.segment_sum(src, seg, n)
class _Rng:
    def __init__(self, key):
        self._k = key
    def _next(self):
        self._k, sub = jax.random.split(self._k)
        return sub
    def normal(self, shape):
        return jax.random.normal(self._next(), shape, dtype=jnp.bfloat16)
    def randint(self, lo, hi, shape):
        return jax.random.randint(self._next(), shape, lo, hi, dtype=jnp.int32)
    def uniform(self, shape, lo=0.0, hi=1.0):
        return jax.random.uniform(self._next(), shape, jnp.bfloat16, lo, hi)
    def permutation(self, n):
        return jax.random.permutation(self._next(), n)


kernel_name = 'interleave_layers__sliding_local_dilated__softmax_full_mha__prompt'

def setup_inputs():
    _rng = _Rng(jax.random.key(int.from_bytes(__import__("os").urandom(4), "little")))
    _w = (lambda a: (lambda t: t.astype(jnp.bfloat16) if jnp.issubdtype(t.dtype, jnp.floating) else t)(jnp.asarray(a)))
    def _A_setup():
        B, S, D = 1, 2048, 512
        return {
            "x": _w((lambda *s: _rng.normal(s) * 0.05)(B, S, D)),
            "wqkv": _w((lambda *s: _rng.normal(s) * 0.05)(D, 3 * D)),
            "wo": _w((lambda *s: _rng.normal(s) * 0.05)(D, D)),
        }
    _A_in = _A_setup()

    def _B_setup():
        B, S, D = 1, 2048, 512
        return {
            "x": _w((lambda *s: _rng.normal(s) * 0.05)(B, S, D)),
            "wqkv": _w((lambda *s: _rng.normal(s) * 0.05)(D, 3 * D)),
            "wo": _w((lambda *s: _rng.normal(s) * 0.05)(D, D)),
        }
    _B_in = _B_setup()

    return {
        "A_x": _A_in["x"],
        "A_wqkv": _A_in["wqkv"],
        "A_wo": _A_in["wo"],
        "B_x": _B_in["x"],
        "B_wqkv": _B_in["wqkv"],
        "B_wo": _B_in["wo"],
    }

def reference(A_x, A_wqkv, A_wo, B_x, B_wqkv, B_wo):
    def _A_ref(x, wqkv, wo):
        B, S, D = x.shape
        H = 32; Dh = D // H
        W, dil = 8, 2
        qkv = (lambda x, *d: x.transpose(*d))((x @ wqkv).reshape(B, S, 3, H, Dh), 2, 0, 3, 1, 4)
        q, k, v = qkv[0], qkv[1], qkv[2]
        scale = Dh ** -0.5
        pos = jnp.arange(S)
        off = jnp.arange(W) * dil
        idx = pos[:, None] - off[None, :]
        mask = idx >= 0
        idx_c = jnp.where(mask, idx, 0).reshape(-1)
        kg = k[:, :, idx_c, :].reshape(B, H, S, W, Dh)
        vg = v[:, :, idx_c, :].reshape(B, H, S, W, Dh)
        logits = jnp.einsum("bhsd,bhswd->bhsw", q, kg) * scale
        logits = jnp.where(mask[None, None, :, :], logits, -1e9)
        attn = _softmax(logits, axis=-1)
        o = jnp.einsum("bhsw,bhswd->bhsd", attn, vg)
        return (lambda x, *d: x.transpose(*d))(o, 0, 2, 1, 3).reshape(B, S, D) @ wo

    def _B_ref(x, wqkv, wo):
        B, S, D = x.shape
        H = 32; Dh = D // H
        qkv = (lambda x, *d: x.transpose(*d))((x @ wqkv).reshape(B, S, 3, H, Dh), 2, 0, 3, 1, 4)
        q, k, v = qkv[0], qkv[1], qkv[2]
        scale = Dh ** -0.5
        scores = jnp.einsum("bhqd,bhkd->bhqk", q, k) * scale
        p = _softmax(scores, axis=-1)
        o = jnp.einsum("bhqk,bhkd->bhqd", p, v)
        return (lambda x, *d: x.transpose(*d))(o, 0, 2, 1, 3).reshape(B, S, D) @ wo

    x = A_x
    x = x + _A_ref(_layernorm(x, axis=-1), A_wqkv, A_wo)
    x = x + _B_ref(_layernorm(x, axis=-1), B_wqkv, B_wo)
    x = x + _A_ref(_layernorm(x, axis=-1), A_wqkv, A_wo)
    x = x + _B_ref(_layernorm(x, axis=-1), B_wqkv, B_wo)
    return x
```

```python
import jax
import jax.numpy as jnp
from jax import lax
from jax.experimental import pallas as pl
from jax.experimental.pallas import tpu as pltpu

S = 2048
D = 512
H = 32
DH = D // H
WIN = 8
LANES = 128
NT = S // LANES
KT = D // LANES
QT = 4
QW = QT * LANES
HEADS_PER_STEP = 4
PV_LAG = 2
EPS = 1e-5
MASKED = -1e9
LOG2E = 1.4426950408889634
QK_SCALE = DH ** -0.5
SUM_LO = 2.0 ** -20
SUM_HI = 2.0 ** 100
ACC_HI = 2.0 ** 120

F32 = jnp.float32
BF16 = jnp.bfloat16
U32 = jnp.uint32


def _lanes(parts):
    return parts[0] if len(parts) == 1 else jnp.concatenate(parts, axis=1)


def _tile(v, t):
    return v[:, t * LANES:(t + 1) * LANES]


def _weight(w_ref, lo, n):
    return _lanes([w_ref[kt, pl.ds(lo, n), :] for kt in range(KT)])


def _kernel(x_hbm, wa_hbm, woa_hbm, wb_hbm, wob_hbm, out_hbm,
            x_in, wa_in, woa_in, wb_in, wob_in, stage_w, stage_x,
            wa_t, woa_t, wb_t, wob_t,
            xt, xn, qa, ka, va, ot, qb, kb, vb, sems):

    copies = [
        pltpu.make_async_copy(src, dst, sems.at[i])
        for i, (src, dst) in enumerate((
            (wa_hbm, wa_in), (x_hbm, x_in), (woa_hbm, woa_in),
            (wb_hbm, wb_in), (wob_hbm, wob_in)))
    ]
    for cp in copies:
        cp.start()

    copies[0].wait()
    for kt in range(KT):
        for cg in range(3 * KT):
            blk = wa_in[kt * LANES:(kt + 1) * LANES, cg * LANES:(cg + 1) * LANES]
            stage_w[kt, cg * LANES:(cg + 1) * LANES, :] = blk.astype(F32).T
    for kt in range(KT):
        for part in range(3):
            for d in range(DH):
                rows = stage_w[kt, pl.ds(part * D + d, H, stride=DH), :]
                wa_t[kt, pl.ds(part * D + d * H, H), :] = rows.astype(BF16)

    copies[1].wait()
    for ft in range(KT):
        stage_x[ft] = pltpu.bitcast(x_in[:, ft * LANES:(ft + 1) * LANES], U32)
    for j in range(NT // 2):
        for ft in range(KT):
            w = stage_x[ft, pl.ds(j, LANES, stride=NT // 2), :].T
            rows = pl.ds(ft * LANES, LANES)
            xt[j, rows, :] = pltpu.bitcast(w << 16, F32)
            xt[NT // 2 + j, rows, :] = pltpu.bitcast(w & jnp.uint32(0xFFFF0000), F32)

    copies[2].wait()
    for ft in range(KT):
        stage_w[ft, 0:D, :] = woa_in[:, ft * LANES:(ft + 1) * LANES].astype(F32)
    for ft in range(KT):
        for ct in range(KT):
            per = LANES // H
            blk = jnp.concatenate(
                [stage_w[ft, pl.ds(ct * per + i, H, stride=DH), :] for i in range(per)], axis=0)
            woa_t[ct, ft * LANES:(ft + 1) * LANES, :] = blk.T.astype(BF16)

    copies[3].wait()
    for kt in range(KT):
        for cg in range(3 * KT):
            blk = wb_in[kt * LANES:(kt + 1) * LANES, cg * LANES:(cg + 1) * LANES]
            wb_t[kt, cg * LANES:(cg + 1) * LANES, :] = blk.astype(F32).T.astype(BF16)
    copies[4].wait()
    for kt in range(KT):
        for cg in range(KT):
            blk = wob_in[kt * LANES:(kt + 1) * LANES, cg * LANES:(cg + 1) * LANES]
            wob_t[kt, cg * LANES:(cg + 1) * LANES, :] = blk.astype(F32).T.astype(BF16)

    def layer_norm(c):
        x = xt[c]
        mean = jnp.sum(x, axis=0, keepdims=True) * (1.0 / D)
        xc = x - mean
        var = jnp.sum(xc * xc, axis=0, keepdims=True) * (1.0 / D)
        xn[c] = (xc * lax.rsqrt(var + EPS)).astype(BF16)

    def project(w_ref, lo, n, src, c0):
        rhs = _lanes([src[c0 + t] for t in range(QT)])
        return jnp.dot(_weight(w_ref, lo, n), rhs, preferred_element_type=F32)

    def out_project(w_ref, c0):
        y = project(w_ref, 0, D, ot, c0)
        for t in range(QT):
            xt[c0 + t] = xt[c0 + t] + _tile(y, t)

    half = NT // 2
    lane = lax.broadcasted_iota(jnp.int32, (8, LANES), 1)

    def a_qkv(par, blk):
        c0 = par * half + blk * QT
        for t in range(QT):
            layer_norm(c0 + t)
        q = project(wa_t, 0, D, xn, c0) * (QK_SCALE * LOG2E)
        k = project(wa_t, D, D, xn, c0)
        v = project(wa_t, 2 * D, D, xn, c0)
        for t in range(QT):
            j = blk * QT + t
            qa[par, j] = _tile(q, t)
            ka[par, half + j] = _tile(k, t)
            va[par, half + j] = _tile(v, t)

    def a_wrap(par):
        first = lax.broadcasted_iota(jnp.int32, (D, LANES), 1) == 0
        for j in range(1, half):
            ka[par, j] = pltpu.roll(ka[par, half + j], 1, 1)
            va[par, j] = jnp.where(first, va[0, half], pltpu.roll(va[par, half + j], 1, 1))

    def a_attend(par, j):
        for hg in range(H // 16):
            outs = []
            for sub in range(2):
                def rows(d):
                    return pl.ds(d * H + hg * 16 + sub * 8, 8)
                logit = [None] * WIN
                for d in range(DH):
                    qd = qa[par, j, rows(d), :]
                    for w in range(WIN):
                        term = qd * ka[par, half + j - w, rows(d), :]
                        logit[w] = term if d == 0 else logit[w] + term
                for w in range(j + 1, WIN):
                    logit[w] = jnp.where(lane == 0, MASKED * LOG2E, logit[w])
                top = logit[0]
                for w in range(1, WIN):
                    top = jnp.maximum(top, logit[w])
                e = [jnp.exp2(lg - top) for lg in logit]
                total = e[0]
                for w in range(1, WIN):
                    total = total + e[w]
                inv = 1.0 / total
                prob = [ew * inv for ew in e]
                res = []
                for d in range(DH):
                    acc = prob[0] * va[par, half + j, rows(d), :]
                    for w in range(1, WIN):
                        acc = acc + prob[w] * va[par, half + j - w, rows(d), :]
                    res.append(acc)
                outs.append(res)
            for d in range(DH):
                pair = jnp.concatenate([outs[0][d], outs[1][d]], axis=0)
                ot[par * half + j, pl.ds(d * H + hg * 16, 16), :] = pair.astype(BF16)

    def b_qkv(c0):
        for t in range(QT):
            layer_norm(c0 + t)
        q = project(wb_t, 0, D, xn, c0) * (QK_SCALE * LOG2E)
        k = project(wb_t, D, D, xn, c0)
        v = project(wb_t, 2 * D, D, xn, c0)
        for t in range(QT):
            qb[c0 + t] = _tile(q, t).astype(BF16)
            vb[c0 + t] = _tile(v, t).astype(BF16)
            for g in range(KT):
                kb[g, c0 + t] = _tile(k, t)[g * LANES:(g + 1) * LANES, :].T.astype(BF16)

    row_head = lax.broadcasted_iota(jnp.int32, (LANES, QW), 0) // DH

    def b_query(h, c0):
        g = h // (LANES // DH)
        g0 = pl.multiple_of(g * LANES, LANES)
        q = _lanes([qb[c0 + t, pl.ds(g0, LANES), :] for t in range(QT)])
        return g, jnp.where(row_head == h % (LANES // DH), q, jnp.zeros_like(q))

    def b_store(h, c0, o):
        r0 = pl.multiple_of(h * DH, DH)
        for t in range(QT):
            ot[c0 + t, pl.ds(r0, DH), :] = _tile(o, t).astype(BF16)

    def b_fast(i, bad):
        per_block = H // HEADS_PER_STEP
        c0 = (i // per_block) * QT
        h0 = (i % per_block) * HEADS_PER_STEP
        acc = [None] * HEADS_PER_STEP
        den = [None] * HEADS_PER_STEP
        pending = []

        def weigh(bad):
            n, c, p = pending.pop(0)
            r0 = pl.multiple_of((h0 + n) * DH, DH)
            part = jnp.dot(vb[c, pl.ds(r0, DH), :], p, preferred_element_type=F32)
            acc[n] = part if c == 0 else acc[n] + part
            if c == NT - 1:
                total = jnp.sum(den[n], axis=0, keepdims=True)
                b_store(h0 + n, c0, acc[n] * (1.0 / total))
                ok = (total >= SUM_LO) & (total <= SUM_HI) & (jnp.abs(acc[n]) <= ACC_HI)
                bad = jnp.where(ok, bad, 1.0)
            return bad

        for n in range(HEADS_PER_STEP):
            g, q = b_query(h0 + n, c0)
            for c in range(NT):
                p = jnp.exp2(jnp.dot(kb[g, c], q, preferred_element_type=F32))
                part = jnp.sum(p.reshape(LANES // 8, 8, QW), axis=0)
                den[n] = part if c == 0 else den[n] + part
                pending.append((n, c, p.astype(BF16)))
                if len(pending) > PV_LAG:
                    bad = weigh(bad)
        while pending:
            bad = weigh(bad)
        return bad

    def b_safe(i, carry):
        c0 = (i // H) * QT
        h = i % H
        g, q = b_query(h, c0)
        r0 = pl.multiple_of(h * DH, DH)

        def step(c, state):
            top, den, acc = state
            s = jnp.dot(kb[g, c], q, preferred_element_type=F32)
            new_top = jnp.maximum(top, jnp.max(s, axis=0, keepdims=True))
            keep = jnp.exp2(top - new_top)
            p = jnp.exp2(s - new_top)
            den = den * keep + jnp.sum(p, axis=0, keepdims=True)
            acc = acc * keep + jnp.dot(vb[c, pl.ds(r0, DH), :], p.astype(BF16),
                                       preferred_element_type=F32)
            return new_top, den, acc

        init = (jnp.full((1, QW), -jnp.inf, F32), jnp.zeros((1, QW), F32),
                jnp.zeros((DH, QW), F32))
        _, den, acc = lax.fori_loop(0, NT, step, init)
        b_store(h, c0, acc / den)
        return carry

    def layer_pair(_, carry):
        def a_front(par, c):
            for blk in range(half // QT):
                a_qkv(par, blk)
            a_wrap(par)
            return c
        lax.fori_loop(0, 2, a_front, 0)

        def a_back(par, c):
            for j in range(half):
                a_attend(par, j)
            for blk in range(half // QT):
                out_project(woa_t, par * half + blk * QT)
            return c
        lax.fori_loop(0, 2, a_back, 0)

        def b_front(blk, c):
            b_qkv(blk * QT)
            return c
        lax.fori_loop(0, NT // QT, b_front, 0)

        bad = lax.fori_loop(0, (NT // QT) * (H // HEADS_PER_STEP), b_fast,
                            jnp.zeros((DH, QW), F32))

        @pl.when(jnp.max(bad) > 0.0)
        def _():
            lax.fori_loop(0, (NT // QT) * H, b_safe, 0)

        def b_back(blk, c):
            out_project(wob_t, blk * QT)
            return c
        lax.fori_loop(0, NT // QT, b_back, 0)
        return carry

    lax.fori_loop(0, 2, layer_pair, 0)

    for j in range(NT // 2):
        for ft in range(KT):
            rows = pl.ds(ft * LANES, LANES)
            even = pltpu.bitcast(xt[j, rows, :].astype(BF16).astype(F32), U32)
            odd = pltpu.bitcast(xt[NT // 2 + j, rows, :].astype(BF16).astype(F32), U32)
            stage_x[ft, pl.ds(j, LANES, stride=NT // 2), :] = ((even >> 16) | odd).T
    for ft in range(KT):
        x_in[:, ft * LANES:(ft + 1) * LANES] = pltpu.bitcast(stage_x[ft], BF16)
    done = pltpu.make_async_copy(x_in, out_hbm, sems.at[0])
    done.start()
    done.wait()


@jax.jit
def pallas_interleave_layers__sliding_local_dilated__softmax_full_mha__prompt_kernel(
    A_x: jax.Array,
    A_wqkv: jax.Array,
    A_wo: jax.Array,
    B_x: jax.Array,
    B_wqkv: jax.Array,
    B_wo: jax.Array,
):
    del B_x
    assert A_x.shape == (1, S, D) and A_x.dtype == BF16
    hbm = pl.BlockSpec(memory_space=pl.ANY)
    out = pl.pallas_call(
        _kernel,
        out_shape=jax.ShapeDtypeStruct((S, D), BF16),
        in_specs=[hbm] * 5,
        out_specs=hbm,
        scratch_shapes=[
            pltpu.VMEM((S, D), BF16),
            pltpu.VMEM((D, 3 * D), BF16),
            pltpu.VMEM((D, D), BF16),
            pltpu.VMEM((D, 3 * D), BF16),
            pltpu.VMEM((D, D), BF16),
            pltpu.VMEM((KT, 3 * D, LANES), F32),
            pltpu.VMEM((KT, S // 2, LANES), U32),
            pltpu.VMEM((KT, 3 * D, LANES), BF16),
            pltpu.VMEM((KT, D, LANES), BF16),
            pltpu.VMEM((KT, 3 * D, LANES), BF16),
            pltpu.VMEM((KT, D, LANES), BF16),
            pltpu.VMEM((NT, D, LANES), F32),
            pltpu.VMEM((NT, D, LANES), BF16),
            pltpu.VMEM((2, NT // 2, D, LANES), F32),
            pltpu.VMEM((2, NT, D, LANES), F32),
            pltpu.VMEM((2, NT, D, LANES), F32),
            pltpu.VMEM((NT, D, LANES), BF16),
            pltpu.VMEM((NT, D, LANES), BF16),
            pltpu.VMEM((KT, NT, LANES, LANES), BF16),
            pltpu.VMEM((NT, D, LANES), BF16),
            pltpu.SemaphoreType.DMA((5,)),
        ],
        compiler_params=pltpu.CompilerParams(vmem_limit_bytes=100 * 1024 * 1024),
    )(A_x.reshape(S, D), A_wqkv, A_wo, B_wqkv, B_wo)
    return out.reshape(1, S, D)
```

```python
from functools import partial, reduce

import jax
import jax.numpy as jnp
from jax import lax
from jax.experimental import pallas as pl
from jax.experimental.pallas import tpu as pltpu

S = 2048
D = 512
H = 32
DH = D // H
WIN = 8
LANES = 128
NT = S // LANES
KT = D // LANES
QT = 4
QW = QT * LANES
NB = NT // QT
GROUP = LANES // DH
VPU_KEYS = 16
MXU_KEYS = LANES - VPU_KEYS
PV_LAG = 2
HEADS_PER_STEP = 2
KEYS_AHEAD = 2
TIE_LAG = 4
ROWS = 256
FINE = 128
EPS = 1e-5
MASKED = -1e9
LOG2E = 1.4426950408889634
QK_SCALE = DH ** -0.5
SUM_LO = 2.0 ** -20
SUM_HI = 2.0 ** 100
ACC_HI = 2.0 ** 120

F32 = jnp.float32
BF16 = jnp.bfloat16
U32 = jnp.uint32


def _lanes(parts):
    return parts[0] if len(parts) == 1 else jnp.concatenate(parts, axis=1)


def _tile(v, t):
    return v[:, t * LANES:(t + 1) * LANES]


def _weave(*streams):
    order = sorted(((i + 0.5) / len(steps), n, i)
                   for n, steps in enumerate(streams) for i in range(len(steps)))
    for _, n, i in order:
        streams[n][i]()


def _kernel(x_hbm, wa_hbm, woa_hbm, wb_hbm, wob_hbm, out_hbm,
            x_io, wa_in, woa_in, wb_in, wob_in, stage_w, stage_x,
            wa_t, woa_t, wb_t, wob_t,
            xt, xn, qa, ka, va, ot, qb, qf, kf, vb, nums, dens, sems, *key_tiles):
    kq, kl = key_tiles[:NT], key_tiles[NT:]

    half = NT // 2
    lane = lax.broadcasted_iota(jnp.int32, (8, LANES), 1)


    def chunk(i):
        return pl.ds(i * LANES, LANES)

    x_loads = [pltpu.make_async_copy(x_hbm.at[:, chunk(i)], x_io.at[i], sems.at[i])
               for i in range(KT)]
    wa_loads = [pltpu.make_async_copy(wa_hbm.at[:, pl.ds(i * D, D)], wa_in.at[i], sems.at[KT + i])
                for i in range(3)]
    late_loads = [pltpu.make_async_copy(src, dst, sems.at[KT + 3 + i]) for i, (src, dst) in
                  enumerate(((woa_hbm, woa_in), (wb_hbm, wb_in), (wob_hbm, wob_in)))]
    for cp in wa_loads[:1] + x_loads:
        cp.start()

    def prepare_wqkv_a(part, kt):
        for cg in range(KT):
            stage_w[kt, chunk(part * KT + cg), :] = wa_in[part, chunk(kt), chunk(cg)].astype(F32).T
        for d in range(DH):
            rows = stage_w[kt, pl.ds(part * D + d, H, stride=DH), :]
            wa_t[kt, pl.ds(part * D + d * H, H), :] = rows.astype(BF16)

    wa_loads[0].wait()
    for kt in range(KT):
        prepare_wqkv_a(0, kt)

    for ft in range(KT):
        x_loads[ft].wait()
        if ft == KT - 2:
            for cp in wa_loads[1:]:
                cp.start()
        if ft == KT - 1:
            for cp in late_loads:
                cp.start()
        stage_x[ft] = pltpu.bitcast(x_io[ft], U32)
        for j in range(half):
            w = stage_x[ft, pl.ds(j, LANES, stride=half), :].T
            xt[j, chunk(ft), :] = pltpu.bitcast(w << 16, F32)
            xt[half + j, chunk(ft), :] = pltpu.bitcast(w & jnp.uint32(0xFFFF0000), F32)

    def prepare_wo_a(ft):
        stage_w[ft, 0:D, :] = woa_in[:, chunk(ft)].astype(F32)
        per = LANES // H
        for ct in range(KT):
            blk = jnp.concatenate(
                [stage_w[ft, pl.ds(ct * per + i, H, stride=DH), :] for i in range(per)], axis=0)
            woa_t[ct, chunk(ft), :] = blk.T.astype(BF16)

    def transpose_weight(src, dst, kt, cg):
        dst[kt, chunk(cg), :] = src[chunk(kt), chunk(cg)].astype(F32).T.astype(BF16)

    def late_weights():
        return ([partial(prepare_wo_a, ft) for ft in range(KT)]
                + [partial(transpose_weight, wb_in, wb_t, kt, cg)
                   for cg in range(3 * KT) for kt in range(KT)]
                + [partial(transpose_weight, wob_in, wob_t, kt, cg)
                   for cg in range(KT) for kt in range(KT)])

    pace = {}

    def paced(v, i):
        y = pace["latest"]
        r = (i * 8) % y.shape[0]
        return jnp.where(pace["never"], y[r:r + 8, :LANES], v)

    def layer_norm(c):
        x = xt[c]
        mean = jnp.sum(x, axis=0, keepdims=True) * (1.0 / D)
        xc = x - mean
        var = jnp.sum(xc * xc, axis=0, keepdims=True) * (1.0 / D)
        scale = lax.rsqrt(var + EPS)
        xn[c] = (xc * scale).astype(BF16)
        pace["never"] = jnp.broadcast_to(scale, (8, LANES)) < 0.0

    def norms(c0):
        return [partial(layer_norm, c0 + t) for t in range(QT)]

    def project(w_ref, lo, n, src, c0):
        w = _lanes([w_ref[kt, pl.ds(lo, n), :] for kt in range(KT)])
        y = jnp.dot(w, _lanes([src[c0 + t] for t in range(QT)]), preferred_element_type=F32)
        pace["latest"] = y
        return y

    def out_project(w_ref, c0, lo, n):
        y = project(w_ref, lo, n, ot, c0)
        for t in range(QT):
            xt[c0 + t, pl.ds(lo, n), :] = xt[c0 + t, pl.ds(lo, n), :] + _tile(y, t)

    def out_steps(w_ref, c0, n=ROWS):
        return [partial(out_project, w_ref, c0, lo, n) for lo in range(0, D, n)]

    def a_qkv(c0, part, lo, n):
        y = project(wa_t, part * D + lo, n, xn, c0)
        rows = pl.ds(lo, n)
        for t in range(QT):
            par, j = divmod(c0 + t, half)
            if part == 0:
                qa[par, j, rows, :] = _tile(y, t) * (QK_SCALE * LOG2E)
                continue
            dst = ka if part == 1 else va
            dst[par, half + j, rows, :] = _tile(y, t)
            if j > 0:
                moved = pltpu.roll(_tile(y, t), 1, 1)
                if part == 2:
                    first = lax.broadcasted_iota(jnp.int32, moved.shape, 1) == 0
                    moved = jnp.where(first, va[0, half, rows, :], moved)
                dst[par, j, rows, :] = moved

    def a_qkv_steps(c0, n=ROWS):
        return [partial(a_qkv, c0, part, lo, n) for part in range(3) for lo in range(0, D, n)]

    def a_attend_steps(par, j, hg):
        logit, prob, res = {}, {}, {}

        def rows(sub, d):
            return pl.ds(d * H + hg * 16 + sub * 8, 8)

        def score(sub, d):
            qd = paced(qa[par, j, rows(sub, d), :], d)
            for w in range(WIN):
                term = qd * ka[par, half + j - w, rows(sub, d), :]
                logit[sub, w] = term if d == 0 else logit[sub, w] + term

        def soften(sub):
            lg = [logit[sub, w] if w <= j else jnp.where(lane == 0, MASKED * LOG2E, logit[sub, w])
                  for w in range(WIN)]
            top = reduce(jnp.maximum, lg)
            e = [jnp.exp2(x - top) for x in lg]
            inv = 1.0 / reduce(jnp.add, e)
            prob[sub] = [x * inv for x in e]

        def mix(sub, d):
            prob[sub] = [paced(prob[sub][0], d)] + prob[sub][1:]
            res[sub, d] = reduce(jnp.add, [prob[sub][w] * va[par, half + j - w, rows(sub, d), :]
                                           for w in range(WIN)])
            if sub == 1:
                pair = jnp.concatenate([res[0, d], res[1, d]], axis=0)
                ot[par * half + j, pl.ds(d * H + hg * 16, 16), :] = pair.astype(BF16)

        steps = []
        for sub in range(2):
            steps += [partial(score, sub, d) for d in range(DH)] + [partial(soften, sub)]
        return steps + [partial(mix, sub, d) for d in range(DH) for sub in range(2)]

    def a_attend(par):
        return [step for j in range(half) for hg in range(H // 16)
                for step in a_attend_steps(par, j, hg)]

    def b_keys(h, c):
        shift = (LANES - (h % GROUP) * DH) % LANES
        return pltpu.roll(kf[h // GROUP, c], shift, 1)

    def spread_keys(h, c):
        keys = b_keys(h, c)
        kq[c][...] = keys.astype(BF16)
        keys = keys[MXU_KEYS:, :]
        for d in range(DH):
            copies = jnp.broadcast_to(keys[:, d:d + 1], keys.shape)
            kl[c][0, d] = copies
            yield copies

    def b_qkv(c0, part, lo, n):
        y = project(wb_t, part * D + lo, n, xn, c0)
        rows = pl.ds(lo, n)
        if part == 0:
            y = y * (QK_SCALE * LOG2E)
            qf[c0 // QT, pl.ds(lo // DH, n // DH)] = y.reshape(n // DH, DH, QW)
        for t in range(QT):
            if part == 1:
                for g in range(n // LANES):
                    kf[lo // LANES + g, c0 + t] = _tile(y, t)[g * LANES:(g + 1) * LANES, :].T
            else:
                (qb if part == 0 else vb)[c0 + t, rows, :] = _tile(y, t).astype(BF16)

    def b_qkv_steps(c0, n=ROWS):
        return [partial(b_qkv, c0, part, lo, n) for part in (1, 0, 2) for lo in range(0, D, n)]

    def b_query(h, c0):
        r0 = pl.multiple_of(h * DH, DH)
        return _lanes([qb[c0 + t, pl.ds(r0, DH), :] for t in range(QT)])

    def normalise(num, den, bad):
        total = jnp.sum(den, axis=0, keepdims=True)
        ok = (total >= SUM_LO) & (total <= SUM_HI) & (jnp.abs(num) <= ACC_HI)
        return (num * (1.0 / total)).astype(BF16), jnp.where(ok, bad, 1.0)

    def head_rows(h):
        return pl.ds(pl.multiple_of(h * DH, DH), DH)

    def b_head(h, n, bad, pending, fetched, zero):
        before, after = jnp.maximum(h - HEADS_PER_STEP, 0), jnp.minimum(h + 1, H - 1)
        acc, den = {}, [None] * NT

        def weigh(blk, c, p):
            part = jnp.dot(vb[c, head_rows(h), :], p, preferred_element_type=F32)
            acc[blk] = part if c == 0 else acc[blk] + part

        def vpu_weights(blk, c, offset, out):
            for r in range(VPU_KEYS // 8):
                s = [None] * QT
                for d in range(DH):
                    kd = kl[c][offset, d, r * 8:(r + 1) * 8, :]
                    for t in range(QT):
                        qd = jnp.broadcast_to(qf[blk, h + offset, d:d + 1, chunk(t)], (8, LANES))
                        s[t] = kd * qd if d == 0 else s[t] + kd * qd
                    if d == DH - 1:
                        out.append([jnp.exp2(st) for st in s])
                    yield

        def add_up(blk, rows):
            for t in range(QT):
                i = blk * QT + t
                for row in rows:
                    den[i] = row[t] if den[i] is None else den[i] + row[t]

        stages = DH * VPU_KEYS // 8
        queries = [b_query(h, blk * QT) for blk in range(NB)]
        for c in range(NT):
            if c + KEYS_AHEAD < NT:
                prefetch = spread_keys(h, c + KEYS_AHEAD)
            else:
                prefetch = spread_keys(after, c + KEYS_AHEAD - NT)
            shared = n > 0 or c > 0
            keys = MXU_KEYS if shared else LANES
            for blk in range(NB):
                s = jnp.dot(kq[c][:keys, :DH], queries[blk], preferred_element_type=F32)
                rows, extra, done = [], [], 0
                side = vpu_weights(blk, c, zero[blk], extra)
                for r in range(keys // 8):
                    rows.append([jnp.exp2(_tile(s, t)[r * 8:(r + 1) * 8, :]) for t in range(QT)])
                    if r % 2 == 1:
                        add_up(blk, rows[-2:])
                    upto = (r + 1) * stages // (keys // 8) if shared else 0
                    for _ in range(done, upto):
                        next(side)
                    done = upto
                    if r % 3 == 2 and r < 12:
                        fetched.append(next(prefetch))
                add_up(blk, extra)
                while len(fetched) > (TIE_LAG if shared else 0):
                    old = fetched.pop(0)
                    if shared:
                        extra[-1][0] = jnp.where(pace["never"], old[8:], extra[-1][0])
                p = jnp.concatenate([_lanes(row) for row in rows + extra], axis=0)
                pending.append(partial(weigh, blk, c, p.astype(BF16)))
                if len(pending) > PV_LAG:
                    pending.pop(0)()
                if blk == 1:
                    done_tile, bad = normalise(nums[n, c], dens[n, c], bad)
                if blk == NB - 1:
                    ot[c, head_rows(before), :] = done_tile
        return bad, acc, den

    def b_fast(i, bad):
        zero = [i // (H + 1 + 2 * blk) for blk in range(NB)]
        pending, fetched, sums = [], [], []
        for n in range(HEADS_PER_STEP):
            bad, acc, den = b_head(i * HEADS_PER_STEP + n, n, bad, pending, fetched, zero)
            sums.append((acc, den))
        for last in pending:
            last()
        for n, (acc, den) in enumerate(sums):
            for c in range(NT):
                nums[n, c], dens[n, c] = _tile(acc[c // QT], c % QT), den[c]
        return bad

    def first_keys(c):
        for _ in spread_keys(0, c):
            pass

    def b_attend():
        nums[...] = jnp.zeros(nums.shape, F32)
        dens[...] = jnp.ones(dens.shape, F32)
        bad = lax.fori_loop(0, H // HEADS_PER_STEP, b_fast, jnp.zeros((DH, LANES), F32))
        for n in range(HEADS_PER_STEP):
            rows = pl.ds((H - HEADS_PER_STEP + n) * DH, DH)
            for c in range(NT):
                ot[c, rows, :], bad = normalise(nums[n, c], dens[n, c], bad)

        @pl.when(jnp.max(bad) > 0.0)
        def _():
            lax.fori_loop(0, (NT // QT) * H, b_safe, 0)

    def b_safe(i, carry):
        c0 = (i // H) * QT
        h = i % H
        r0 = pl.multiple_of(h * DH, DH)
        q = b_query(h, c0)

        def step(c, state):
            top, den, acc = state
            keys = b_keys(h, c)[:, :DH].astype(BF16)
            s = jnp.dot(keys, q, preferred_element_type=F32)
            new_top = jnp.maximum(top, jnp.max(s, axis=0, keepdims=True))
            keep = jnp.exp2(top - new_top)
            p = jnp.exp2(s - new_top)
            den = den * keep + jnp.sum(p, axis=0, keepdims=True)
            acc = acc * keep + jnp.dot(vb[c, pl.ds(r0, DH), :], p.astype(BF16),
                                       preferred_element_type=F32)
            return new_top, den, acc

        init = (jnp.full((1, QW), -jnp.inf, F32), jnp.zeros((1, QW), F32),
                jnp.zeros((DH, QW), F32))
        _, den, acc = lax.fori_loop(0, NT, step, init)
        out = acc / den
        for t in range(QT):
            ot[c0 + t, pl.ds(r0, DH), :] = _tile(out, t).astype(BF16)
        return carry

    for pair in range(2):
        if pair == 0:
            _weave(norms(0))
            first, second = a_qkv_steps(0), a_qkv_steps(QT)
            n = len(first) // 3
            _weave(first[:n], norms(QT))
            wa_loads[1].wait()
            wa_loads[2].wait()
            _weave(second[:n], [partial(prepare_wqkv_a, 1, kt) for kt in range(KT)])
            _weave(first[n:2 * n] + second[n:2 * n],
                   [partial(prepare_wqkv_a, 2, kt) for kt in range(KT)])
            _weave(first[2 * n:] + second[2 * n:], norms(2 * QT) + norms(3 * QT))
        else:
            _weave(out_steps(wob_t, 0))
            _weave(out_steps(wob_t, QT) + out_steps(wob_t, 2 * QT) + out_steps(wob_t, 3 * QT),
                   norms(0) + norms(QT))
            _weave(a_qkv_steps(0) + a_qkv_steps(QT), norms(2 * QT) + norms(3 * QT))
        extra = []
        if pair == 0:
            for cp in late_loads:
                cp.wait()
            extra = late_weights()
        _weave(a_qkv_steps(2 * QT, FINE) + a_qkv_steps(3 * QT, FINE), a_attend(0), extra)
        _weave(out_steps(woa_t, 0, FINE) + out_steps(woa_t, QT, FINE) + norms(0) + norms(QT)
               + b_qkv_steps(0, FINE) + b_qkv_steps(QT, FINE), a_attend(1))
        _weave(out_steps(woa_t, 2 * QT))
        _weave(out_steps(woa_t, 3 * QT), norms(2 * QT))
        _weave(b_qkv_steps(2 * QT), norms(3 * QT),
               [partial(first_keys, c) for c in range(KEYS_AHEAD)])
        _weave(b_qkv_steps(3 * QT))
        b_attend()

    stores = [pltpu.make_async_copy(x_io.at[i], out_hbm.at[:, chunk(i)], sems.at[i])
              for i in range(KT)]

    def store_tile(ft, j):
        even = pltpu.bitcast(xt[j, chunk(ft), :].astype(BF16).astype(F32), U32)
        odd = pltpu.bitcast(xt[half + j, chunk(ft), :].astype(BF16).astype(F32), U32)
        stage_x[ft, pl.ds(j, LANES, stride=half), :] = ((even >> 16) | odd).T

    for ft in range(KT + 1):
        last = [partial(out_project, wob_t, c0, ft * LANES, LANES)
                for c0 in range(0, NT, QT)] if ft < KT else []
        _weave(last, [partial(store_tile, ft - 1, j) for j in range(half)] if ft > 0 else [])
        if ft > 0:
            x_io[ft - 1] = pltpu.bitcast(stage_x[ft - 1], BF16)
            stores[ft - 1].start()
    for cp in stores:
        cp.wait()


@jax.jit
def pallas_interleave_layers__sliding_local_dilated__softmax_full_mha__prompt_kernel(
    A_x: jax.Array,
    A_wqkv: jax.Array,
    A_wo: jax.Array,
    B_x: jax.Array,
    B_wqkv: jax.Array,
    B_wo: jax.Array,
):
    del B_x
    assert A_x.shape == (1, S, D) and A_x.dtype == BF16
    hbm = pl.BlockSpec(memory_space=pl.ANY)
    out = pl.pallas_call(
        _kernel,
        out_shape=jax.ShapeDtypeStruct((S, D), BF16),
        in_specs=[hbm] * 5,
        out_specs=hbm,
        scratch_shapes=[
            pltpu.VMEM((KT, S, LANES), BF16),
            pltpu.VMEM((3, D, D), BF16),
            pltpu.VMEM((D, D), BF16),
            pltpu.VMEM((D, 3 * D), BF16),
            pltpu.VMEM((D, D), BF16),
            pltpu.VMEM((KT, 3 * D, LANES), F32),
            pltpu.VMEM((KT, S // 2, LANES), U32),
            pltpu.VMEM((KT, 3 * D, LANES), BF16),
            pltpu.VMEM((KT, D, LANES), BF16),
            pltpu.VMEM((KT, 3 * D, LANES), BF16),
            pltpu.VMEM((KT, D, LANES), BF16),
            pltpu.VMEM((NT, D, LANES), F32),
            pltpu.VMEM((NT, D, LANES), BF16),
            pltpu.VMEM((2, NT // 2, D, LANES), F32),
            pltpu.VMEM((2, NT, D, LANES), F32),
            pltpu.VMEM((2, NT, D, LANES), F32),
            pltpu.VMEM((NT, D, LANES), BF16),
            pltpu.VMEM((NT, D, LANES), BF16),
            pltpu.VMEM((NT // QT, H, DH, QW), F32),
            pltpu.VMEM((KT, NT, LANES, LANES), F32),
            pltpu.VMEM((NT, D, LANES), BF16),
            pltpu.VMEM((HEADS_PER_STEP, NT, DH, LANES), F32),
            pltpu.VMEM((HEADS_PER_STEP, NT, 8, LANES), F32),
            pltpu.SemaphoreType.DMA((KT + 6,)),
            *[pltpu.VMEM((LANES, LANES), BF16)] * NT,
            *[pltpu.VMEM((1, DH, VPU_KEYS, LANES), F32)] * NT,
        ],
        compiler_params=pltpu.CompilerParams(vmem_limit_bytes=100 * 1024 * 1024),
    )(A_x.reshape(S, D), A_wqkv, A_wo, B_wqkv, B_wo)
    return out.reshape(1, S, D)
```

```python
from functools import partial, reduce

import jax
import jax.numpy as jnp
from jax import lax
from jax.experimental import pallas as pl
from jax.experimental.pallas import tpu as pltpu

S = 2048
D = 512
H = 32
DH = D // H
WIN = 8
LANES = 128
NT = S // LANES
KT = D // LANES
QT = 4
QW = QT * LANES
NB = NT // QT
GROUP = LANES // DH
VPU_KEYS = 16
MXU_KEYS = LANES - VPU_KEYS
PV_LAG = 2
HEADS_PER_STEP = 4
KEYS_AHEAD = 2
TIE_LAG = 6
ROWS = 256
FINE = 128
EPS = 1e-5
MASKED = -1e9
LOG2E = 1.4426950408889634
QK_SCALE = DH ** -0.5
SUM_LO = 2.0 ** -20
SUM_HI = 2.0 ** 100
ACC_HI = 2.0 ** 120

F32 = jnp.float32
BF16 = jnp.bfloat16
U32 = jnp.uint32


def _lanes(parts):
    return parts[0] if len(parts) == 1 else jnp.concatenate(parts, axis=1)


def _tile(v, t):
    return v[:, t * LANES:(t + 1) * LANES]


def _weave(*streams):
    order = sorted(((i + 0.5) / len(steps), n, i)
                   for n, steps in enumerate(streams) for i in range(len(steps)))
    for _, n, i in order:
        streams[n][i]()


def _kernel(x_hbm, wa_hbm, woa_hbm, wb_hbm, wob_hbm, out_hbm,
            x_io, wa_in, woa_in, wb_in, wob_in, stage_w, stage_x,
            wa_t, woa_t, wb_t, wob_t,
            xt, xn, qa, ka, va, ot, qb, qf, kf, vb, nums, dens, sems, *key_tiles):
    kq, kl = key_tiles[:NT], key_tiles[NT:]

    half = NT // 2
    lane = lax.broadcasted_iota(jnp.int32, (8, LANES), 1)


    def chunk(i):
        return pl.ds(i * LANES, LANES)

    x_loads = [pltpu.make_async_copy(x_hbm.at[:, chunk(i)], x_io.at[i], sems.at[i])
               for i in range(KT)]
    wa_loads = [pltpu.make_async_copy(wa_hbm.at[:, pl.ds(i * D, D)], wa_in.at[i], sems.at[KT + i])
                for i in range(3)]
    late_loads = [pltpu.make_async_copy(src, dst, sems.at[KT + 3 + i]) for i, (src, dst) in
                  enumerate(((woa_hbm, woa_in), (wb_hbm, wb_in), (wob_hbm, wob_in)))]
    for cp in wa_loads[:1] + x_loads:
        cp.start()

    def prepare_wqkv_a(part, kt):
        for cg in range(KT):
            stage_w[kt, chunk(part * KT + cg), :] = wa_in[part, chunk(kt), chunk(cg)].astype(F32).T
        for d in range(DH):
            rows = stage_w[kt, pl.ds(part * D + d, H, stride=DH), :]
            wa_t[kt, pl.ds(part * D + d * H, H), :] = rows.astype(BF16)

    wa_loads[0].wait()
    for kt in range(KT):
        prepare_wqkv_a(0, kt)

    for ft in range(KT):
        x_loads[ft].wait()
        if ft == KT - 2:
            for cp in wa_loads[1:]:
                cp.start()
        if ft == KT - 1:
            for cp in late_loads:
                cp.start()
        stage_x[ft] = pltpu.bitcast(x_io[ft], U32)
        for j in range(half):
            w = stage_x[ft, pl.ds(j, LANES, stride=half), :].T
            xt[j, chunk(ft), :] = pltpu.bitcast(w << 16, F32)
            xt[half + j, chunk(ft), :] = pltpu.bitcast(w & jnp.uint32(0xFFFF0000), F32)

    def prepare_wo_a(ft):
        stage_w[ft, 0:D, :] = woa_in[:, chunk(ft)].astype(F32)
        per = LANES // H
        for ct in range(KT):
            blk = jnp.concatenate(
                [stage_w[ft, pl.ds(ct * per + i, H, stride=DH), :] for i in range(per)], axis=0)
            woa_t[ct, chunk(ft), :] = blk.T.astype(BF16)

    def transpose_weight(src, dst, kt, cg):
        dst[kt, chunk(cg), :] = src[chunk(kt), chunk(cg)].astype(F32).T.astype(BF16)

    def late_weights():
        return ([partial(prepare_wo_a, ft) for ft in range(KT)]
                + [partial(transpose_weight, wb_in, wb_t, kt, cg)
                   for cg in range(3 * KT) for kt in range(KT)]
                + [partial(transpose_weight, wob_in, wob_t, kt, cg)
                   for cg in range(KT) for kt in range(KT)])

    pace = {}

    def paced(v, i):
        y = pace["latest"]
        r = (i * 8) % y.shape[0]
        return jnp.where(pace["never"], y[r:r + 8, :LANES], v)

    def layer_norm(c):
        x = xt[c]
        mean = jnp.sum(x, axis=0, keepdims=True) * (1.0 / D)
        xc = x - mean
        var = jnp.sum(xc * xc, axis=0, keepdims=True) * (1.0 / D)
        scale = lax.rsqrt(var + EPS)
        xn[c] = (xc * scale).astype(BF16)
        pace["never"] = jnp.broadcast_to(scale, (8, LANES)) < 0.0

    def norms(c0):
        return [partial(layer_norm, c0 + t) for t in range(QT)]

    def project(w_ref, lo, n, src, c0):
        w = _lanes([w_ref[kt, pl.ds(lo, n), :] for kt in range(KT)])
        y = jnp.dot(w, _lanes([src[c0 + t] for t in range(QT)]), preferred_element_type=F32)
        pace["latest"] = y
        return y

    def out_project(w_ref, c0, lo, n):
        y = project(w_ref, lo, n, ot, c0)
        for t in range(QT):
            xt[c0 + t, pl.ds(lo, n), :] = xt[c0 + t, pl.ds(lo, n), :] + _tile(y, t)

    def out_steps(w_ref, c0, n=ROWS):
        return [partial(out_project, w_ref, c0, lo, n) for lo in range(0, D, n)]

    def a_qkv(c0, part, lo, n):
        y = project(wa_t, part * D + lo, n, xn, c0)
        rows = pl.ds(lo, n)
        for t in range(QT):
            par, j = divmod(c0 + t, half)
            if part == 0:
                qa[par, j, rows, :] = _tile(y, t) * (QK_SCALE * LOG2E)
                continue
            dst = ka if part == 1 else va
            dst[par, half + j, rows, :] = _tile(y, t)
            if j > 0:
                moved = pltpu.roll(_tile(y, t), 1, 1)
                if part == 2:
                    first = lax.broadcasted_iota(jnp.int32, moved.shape, 1) == 0
                    moved = jnp.where(first, va[0, half, rows, :], moved)
                dst[par, j, rows, :] = moved

    def a_qkv_steps(c0, n=ROWS):
        return [partial(a_qkv, c0, part, lo, n) for part in range(3) for lo in range(0, D, n)]

    def a_attend_steps(par, j, hg):
        logit, prob, res = {}, {}, {}

        def rows(sub, d):
            return pl.ds(d * H + hg * 16 + sub * 8, 8)

        def score(sub, d):
            qd = paced(qa[par, j, rows(sub, d), :], d)
            for w in range(WIN):
                term = qd * ka[par, half + j - w, rows(sub, d), :]
                logit[sub, w] = term if d == 0 else logit[sub, w] + term

        def soften(sub):
            lg = [logit[sub, w] if w <= j else jnp.where(lane == 0, MASKED * LOG2E, logit[sub, w])
                  for w in range(WIN)]
            top = reduce(jnp.maximum, lg)
            e = [jnp.exp2(x - top) for x in lg]
            inv = 1.0 / reduce(jnp.add, e)
            prob[sub] = [x * inv for x in e]

        def mix(sub, d):
            prob[sub] = [paced(prob[sub][0], d)] + prob[sub][1:]
            res[sub, d] = reduce(jnp.add, [prob[sub][w] * va[par, half + j - w, rows(sub, d), :]
                                           for w in range(WIN)])
            if sub == 1:
                pair = jnp.concatenate([res[0, d], res[1, d]], axis=0)
                ot[par * half + j, pl.ds(d * H + hg * 16, 16), :] = pair.astype(BF16)

        steps = []
        for sub in range(2):
            steps += [partial(score, sub, d) for d in range(DH)] + [partial(soften, sub)]
        return steps + [partial(mix, sub, d) for d in range(DH) for sub in range(2)]

    def a_attend(par):
        return [step for j in range(half) for hg in range(H // 16)
                for step in a_attend_steps(par, j, hg)]

    def b_keys(h, c):
        shift = (LANES - (h % GROUP) * DH) % LANES
        return pltpu.roll(kf[h // GROUP, c], shift, 1)

    def spread_keys(h, c):
        keys = b_keys(h, c)
        kq[c][...] = keys.astype(BF16)
        keys = keys[MXU_KEYS:, :]
        for d in range(DH):
            copies = jnp.broadcast_to(keys[:, d:d + 1], keys.shape)
            kl[c][0, d] = copies
            yield copies

    def b_qkv(c0, part, lo, n):
        y = project(wb_t, part * D + lo, n, xn, c0)
        rows = pl.ds(lo, n)
        if part == 0:
            y = y * (QK_SCALE * LOG2E)
            qf[c0 // QT, pl.ds(lo // DH, n // DH)] = y.reshape(n // DH, DH, QW)
        for t in range(QT):
            if part == 1:
                for g in range(n // LANES):
                    kf[lo // LANES + g, c0 + t] = _tile(y, t)[g * LANES:(g + 1) * LANES, :].T
            else:
                (qb if part == 0 else vb)[c0 + t, rows, :] = _tile(y, t).astype(BF16)

    def b_qkv_steps(c0, n=ROWS):
        return [partial(b_qkv, c0, part, lo, n) for part in (1, 0, 2) for lo in range(0, D, n)]

    def b_query(h, c0):
        r0 = pl.multiple_of(h * DH, DH)
        return _lanes([qb[c0 + t, pl.ds(r0, DH), :] for t in range(QT)])

    def normalise(num, den, bad):
        total = jnp.sum(den, axis=0, keepdims=True)
        ok = (total >= SUM_LO) & (total <= SUM_HI) & (jnp.abs(num) <= ACC_HI)
        return (num * (1.0 / total)).astype(BF16), jnp.where(ok, bad, 1.0)

    def head_rows(h):
        return pl.ds(pl.multiple_of(h * DH, DH), DH)

    def b_head(h, n, bad, pending, fetched, zero, sums):
        before, after = jnp.maximum(h - HEADS_PER_STEP, 0), jnp.minimum(h + 1, H - 1)
        acc, den = {}, [None] * NT

        def weigh(blk, c, p):
            part = jnp.dot(vb[c, head_rows(h), :], p, preferred_element_type=F32)
            if c == 0 and n > 0:
                never = jnp.tile(pace["never"].astype(jnp.int32), (DH // 8, QT)) > 0
                part = jnp.where(never, sums[n - 1][0][blk], part)
            acc[blk] = part if c == 0 else acc[blk] + part

        def vpu_weights(blk, c, offset, out):
            for r in range(VPU_KEYS // 8):
                s = [None] * QT
                for d in range(DH):
                    kd = kl[c][offset, d, r * 8:(r + 1) * 8, :]
                    for t in range(QT):
                        qd = jnp.broadcast_to(qf[blk, h + offset, d:d + 1, chunk(t)], (8, LANES))
                        s[t] = kd * qd if d == 0 else s[t] + kd * qd
                    if d == DH - 1:
                        out.append([jnp.exp2(st) for st in s])
                    yield

        def add_up(blk, rows):
            for t in range(QT):
                i = blk * QT + t
                for row in rows:
                    den[i] = row[t] if den[i] is None else den[i] + row[t]

        stages = DH * VPU_KEYS // 8
        queries = [b_query(h, blk * QT) for blk in range(NB)]
        for c in range(NT):
            if c + KEYS_AHEAD < NT:
                prefetch = spread_keys(h, c + KEYS_AHEAD)
            else:
                prefetch = spread_keys(after, c + KEYS_AHEAD - NT)
            shared = n > 0 or c > 0
            keys = MXU_KEYS if shared else LANES
            for blk in range(NB):
                s = jnp.dot(kq[c][:keys, :DH], queries[blk], preferred_element_type=F32)
                rows, extra, done = [], [], 0
                side = vpu_weights(blk, c, zero[blk], extra)
                for r in range(keys // 8):
                    rows.append([jnp.exp2(_tile(s, t)[r * 8:(r + 1) * 8, :]) for t in range(QT)])
                    if r % 2 == 1:
                        add_up(blk, rows[-2:])
                    upto = (r + 1) * stages // (keys // 8) if shared else 0
                    for _ in range(done, upto):
                        next(side)
                    done = upto
                    if r % 3 == 2 and r < 12:
                        fetched.append(next(prefetch))
                add_up(blk, extra)
                while len(fetched) > (TIE_LAG if shared else 0):
                    old = fetched.pop(0)
                    if shared and len(fetched) == TIE_LAG:
                        extra[-1][0] = jnp.where(pace["never"], old[8:], extra[-1][0])
                p = jnp.concatenate([_lanes(row) for row in rows + extra], axis=0)
                pending.append(partial(weigh, blk, c, p.astype(BF16)))
                if len(pending) > PV_LAG:
                    pending.pop(0)()
                if blk == 1:
                    done_tile, bad = normalise(nums[n, c], dens[n, c], bad)
                if blk == NB - 1:
                    ot[c, head_rows(before), :] = done_tile
        return bad, acc, den

    def b_fast(i, bad):
        zero = [i // (H + 1 + 2 * blk) for blk in range(NB)]
        pending, fetched, sums = [], [], []
        for n in range(HEADS_PER_STEP):
            bad, acc, den = b_head(i * HEADS_PER_STEP + n, n, bad, pending, fetched, zero, sums)
            sums.append((acc, den))
        for last in pending:
            last()
        for n, (acc, den) in enumerate(sums):
            for c in range(NT):
                nums[n, c], dens[n, c] = _tile(acc[c // QT], c % QT), den[c]
        return bad

    def first_keys(c):
        for _ in spread_keys(0, c):
            pass

    def b_attend():
        nums[...] = jnp.zeros(nums.shape, F32)
        dens[...] = jnp.ones(dens.shape, F32)
        bad = lax.fori_loop(0, H // HEADS_PER_STEP, b_fast, jnp.zeros((DH, LANES), F32))
        for n in range(HEADS_PER_STEP):
            rows = pl.ds((H - HEADS_PER_STEP + n) * DH, DH)
            for c in range(NT):
                ot[c, rows, :], bad = normalise(nums[n, c], dens[n, c], bad)

        @pl.when(jnp.max(bad) > 0.0)
        def _():
            lax.fori_loop(0, (NT // QT) * H, b_safe, 0)

    def b_safe(i, carry):
        c0 = (i // H) * QT
        h = i % H
        r0 = pl.multiple_of(h * DH, DH)
        q = b_query(h, c0)

        def step(c, state):
            top, den, acc = state
            keys = b_keys(h, c)[:, :DH].astype(BF16)
            s = jnp.dot(keys, q, preferred_element_type=F32)
            new_top = jnp.maximum(top, jnp.max(s, axis=0, keepdims=True))
            keep = jnp.exp2(top - new_top)
            p = jnp.exp2(s - new_top)
            den = den * keep + jnp.sum(p, axis=0, keepdims=True)
            acc = acc * keep + jnp.dot(vb[c, pl.ds(r0, DH), :], p.astype(BF16),
                                       preferred_element_type=F32)
            return new_top, den, acc

        init = (jnp.full((1, QW), -jnp.inf, F32), jnp.zeros((1, QW), F32),
                jnp.zeros((DH, QW), F32))
        _, den, acc = lax.fori_loop(0, NT, step, init)
        out = acc / den
        for t in range(QT):
            ot[c0 + t, pl.ds(r0, DH), :] = _tile(out, t).astype(BF16)
        return carry

    for pair in range(2):
        if pair == 0:
            _weave(norms(0))
            first, second = a_qkv_steps(0), a_qkv_steps(QT)
            n = len(first) // 3
            _weave(first[:n], norms(QT))
            wa_loads[1].wait()
            wa_loads[2].wait()
            _weave(second[:n], [partial(prepare_wqkv_a, 1, kt) for kt in range(KT)])
            _weave(first[n:2 * n] + second[n:2 * n],
                   [partial(prepare_wqkv_a, 2, kt) for kt in range(KT)])
            _weave(first[2 * n:] + second[2 * n:], norms(2 * QT) + norms(3 * QT))
        else:
            _weave(out_steps(wob_t, 0))
            _weave(out_steps(wob_t, QT) + out_steps(wob_t, 2 * QT) + out_steps(wob_t, 3 * QT),
                   norms(0) + norms(QT))
            _weave(a_qkv_steps(0) + a_qkv_steps(QT), norms(2 * QT) + norms(3 * QT))
        extra = []
        if pair == 0:
            for cp in late_loads:
                cp.wait()
            extra = late_weights()
        _weave(a_qkv_steps(2 * QT, FINE) + a_qkv_steps(3 * QT, FINE), a_attend(0), extra)
        _weave(out_steps(woa_t, 0, FINE) + out_steps(woa_t, QT, FINE) + norms(0) + norms(QT)
               + b_qkv_steps(0, FINE) + b_qkv_steps(QT, FINE), a_attend(1))
        _weave(out_steps(woa_t, 2 * QT))
        _weave(out_steps(woa_t, 3 * QT), norms(2 * QT))
        _weave(b_qkv_steps(2 * QT), norms(3 * QT),
               [partial(first_keys, c) for c in range(KEYS_AHEAD)])
        _weave(b_qkv_steps(3 * QT))
        b_attend()

    stores = [pltpu.make_async_copy(x_io.at[i], out_hbm.at[:, chunk(i)], sems.at[i])
              for i in range(KT)]

    def store_tile(ft, j):
        even = pltpu.bitcast(xt[j, chunk(ft), :].astype(BF16).astype(F32), U32)
        odd = pltpu.bitcast(xt[half + j, chunk(ft), :].astype(BF16).astype(F32), U32)
        stage_x[ft, pl.ds(j, LANES, stride=half), :] = ((even >> 16) | odd).T

    for ft in range(KT + 1):
        last = [partial(out_project, wob_t, c0, ft * LANES, LANES)
                for c0 in range(0, NT, QT)] if ft < KT else []
        _weave(last, [partial(store_tile, ft - 1, j) for j in range(half)] if ft > 0 else [])
        if ft > 0:
            x_io[ft - 1] = pltpu.bitcast(stage_x[ft - 1], BF16)
            stores[ft - 1].start()
    for cp in stores:
        cp.wait()


@jax.jit
def pallas_interleave_layers__sliding_local_dilated__softmax_full_mha__prompt_kernel(
    A_x: jax.Array,
    A_wqkv: jax.Array,
    A_wo: jax.Array,
    B_x: jax.Array,
    B_wqkv: jax.Array,
    B_wo: jax.Array,
):
    del B_x
    assert A_x.shape == (1, S, D) and A_x.dtype == BF16
    hbm = pl.BlockSpec(memory_space=pl.ANY)
    out = pl.pallas_call(
        _kernel,
        out_shape=jax.ShapeDtypeStruct((S, D), BF16),
        in_specs=[hbm] * 5,
        out_specs=hbm,
        scratch_shapes=[
            pltpu.VMEM((KT, S, LANES), BF16),
            pltpu.VMEM((3, D, D), BF16),
            pltpu.VMEM((D, D), BF16),
            pltpu.VMEM((D, 3 * D), BF16),
            pltpu.VMEM((D, D), BF16),
            pltpu.VMEM((KT, 3 * D, LANES), F32),
            pltpu.VMEM((KT, S // 2, LANES), U32),
            pltpu.VMEM((KT, 3 * D, LANES), BF16),
            pltpu.VMEM((KT, D, LANES), BF16),
            pltpu.VMEM((KT, 3 * D, LANES), BF16),
            pltpu.VMEM((KT, D, LANES), BF16),
            pltpu.VMEM((NT, D, LANES), F32),
            pltpu.VMEM((NT, D, LANES), BF16),
            pltpu.VMEM((2, NT // 2, D, LANES), F32),
            pltpu.VMEM((2, NT, D, LANES), F32),
            pltpu.VMEM((2, NT, D, LANES), F32),
            pltpu.VMEM((NT, D, LANES), BF16),
            pltpu.VMEM((NT, D, LANES), BF16),
            pltpu.VMEM((NT // QT, H, DH, QW), F32),
            pltpu.VMEM((KT, NT, LANES, LANES), F32),
            pltpu.VMEM((NT, D, LANES), BF16),
            pltpu.VMEM((HEADS_PER_STEP, NT, DH, LANES), F32),
            pltpu.VMEM((HEADS_PER_STEP, NT, 8, LANES), F32),
            pltpu.SemaphoreType.DMA((KT + 6,)),
            *[pltpu.VMEM((LANES, LANES), BF16)] * NT,
            *[pltpu.VMEM((1, DH, VPU_KEYS, LANES), F32)] * NT,
        ],
        compiler_params=pltpu.CompilerParams(vmem_limit_bytes=100 * 1024 * 1024),
    )(A_x.reshape(S, D), A_wqkv, A_wo, B_wqkv, B_wo)
    return out.reshape(1, S, D)
```

```python
from functools import partial, reduce

import jax
import jax.numpy as jnp
from jax import lax
from jax.experimental import pallas as pl
from jax.experimental.pallas import tpu as pltpu

S = 2048
D = 512
H = 32
DH = D // H
WIN = 8
LANES = 128
NT = S // LANES
KT = D // LANES
QT = 4
QW = QT * LANES
NB = NT // QT
GROUP = LANES // DH
VPU_KEYS = 16
MXU_KEYS = LANES - VPU_KEYS
PV_LAG = 2
HEADS_PER_STEP = 4
KEYS_AHEAD = 2
TIE_LAG = 6
ROWS = 256
EPS = 1e-5
MASKED = -1e9
LOG2E = 1.4426950408889634
QK_SCALE = DH ** -0.5
SUM_LO = 2.0 ** -20
SUM_HI = 2.0 ** 100
ACC_HI = 2.0 ** 120

F32 = jnp.float32
BF16 = jnp.bfloat16
U32 = jnp.uint32


def _lanes(parts):
    return parts[0] if len(parts) == 1 else jnp.concatenate(parts, axis=1)


def _tile(v, t):
    return v[:, t * LANES:(t + 1) * LANES]


def _weave(*streams):
    order = sorted(((i + 0.5) / len(steps), n, i)
                   for n, steps in enumerate(streams) for i in range(len(steps)))
    for _, n, i in order:
        streams[n][i]()


def _kernel(x_hbm, wa_hbm, woa_hbm, wb_hbm, wob_hbm, out_hbm,
            x_io, wa_in, woa_in, wb_in, wob_in, stage_w, stage_x,
            wa_t, woa_t, wb_t, wob_t,
            xt, xn, qa, ka, va, ot, qb, qf, kf, vb, nums, dens, sems, *key_tiles):
    kq, kl = key_tiles[:NT], key_tiles[NT:]

    half = NT // 2
    lane = lax.broadcasted_iota(jnp.int32, (8, LANES), 1)


    def chunk(i):
        return pl.ds(i * LANES, LANES)

    x_loads = [pltpu.make_async_copy(x_hbm.at[:, chunk(i)], x_io.at[i], sems.at[i])
               for i in range(KT)]
    wa_loads = [pltpu.make_async_copy(wa_hbm.at[:, pl.ds(i * D, D)], wa_in.at[i], sems.at[KT + i])
                for i in range(3)]
    late_loads = [pltpu.make_async_copy(src, dst, sems.at[KT + 3 + i]) for i, (src, dst) in
                  enumerate(((woa_hbm, woa_in), (wb_hbm, wb_in), (wob_hbm, wob_in)))]
    for cp in wa_loads[:1] + x_loads:
        cp.start()

    def prepare_wqkv_a(part, kt):
        for cg in range(KT):
            stage_w[kt, chunk(part * KT + cg), :] = wa_in[part, chunk(kt), chunk(cg)].astype(F32).T
        for d in range(DH):
            rows = stage_w[kt, pl.ds(part * D + d, H, stride=DH), :]
            wa_t[kt, pl.ds(part * D + d * H, H), :] = rows.astype(BF16)

    wa_loads[0].wait()
    for kt in range(KT):
        prepare_wqkv_a(0, kt)

    for ft in range(KT):
        x_loads[ft].wait()
        if ft == KT - 2:
            for cp in wa_loads[1:]:
                cp.start()
        if ft == KT - 1:
            for cp in late_loads:
                cp.start()
        stage_x[ft] = pltpu.bitcast(x_io[ft], U32)
        for j in range(half):
            w = stage_x[ft, pl.ds(j, LANES, stride=half), :].T
            xt[j, chunk(ft), :] = pltpu.bitcast(w << 16, F32)
            xt[half + j, chunk(ft), :] = pltpu.bitcast(w & jnp.uint32(0xFFFF0000), F32)

    def prepare_wo_a(ft):
        stage_w[ft, 0:D, :] = woa_in[:, chunk(ft)].astype(F32)
        per = LANES // H
        for ct in range(KT):
            blk = jnp.concatenate(
                [stage_w[ft, pl.ds(ct * per + i, H, stride=DH), :] for i in range(per)], axis=0)
            woa_t[ct, chunk(ft), :] = blk.T.astype(BF16)

    def transpose_weight(src, dst, kt, cg):
        dst[kt, chunk(cg), :] = src[chunk(kt), chunk(cg)].astype(F32).T.astype(BF16)

    def late_weights():
        return ([partial(prepare_wo_a, ft) for ft in range(KT)]
                + [partial(transpose_weight, wb_in, wb_t, kt, cg)
                   for cg in range(3 * KT) for kt in range(KT)]
                + [partial(transpose_weight, wob_in, wob_t, kt, cg)
                   for cg in range(KT) for kt in range(KT)])

    pace = {}

    def paced(v, i):
        y = pace["latest"]
        r = i * (y.shape[0] // DH)
        return jnp.where(pace["never"], y[r:r + 8, :LANES], v)

    def layer_norm(c):
        x = xt[c]
        mean = jnp.sum(x, axis=0, keepdims=True) * (1.0 / D)
        xc = x - mean
        var = jnp.sum(xc * xc, axis=0, keepdims=True) * (1.0 / D)
        scale = lax.rsqrt(var + EPS)
        xn[c] = (xc * scale).astype(BF16)
        pace["never"] = jnp.broadcast_to(scale, (8, LANES)) < 0.0

    def norms(c0):
        return [partial(layer_norm, c0 + t) for t in range(QT)]

    def project(w_ref, lo, n, src, c0):
        w = _lanes([w_ref[kt, pl.ds(lo, n), :] for kt in range(KT)])
        y = jnp.dot(w, _lanes([src[c0 + t] for t in range(QT)]), preferred_element_type=F32)
        pace["latest"] = y
        return y

    def out_project(w_ref, c0, lo, n):
        y = project(w_ref, lo, n, ot, c0)
        for t in range(QT):
            xt[c0 + t, pl.ds(lo, n), :] = xt[c0 + t, pl.ds(lo, n), :] + _tile(y, t)

    def out_steps(w_ref, c0, n=ROWS):
        return [partial(out_project, w_ref, c0, lo, n) for lo in range(0, D, n)]

    def a_qkv(c0, part, lo, n):
        y = project(wa_t, part * D + lo, n, xn, c0)
        rows = pl.ds(lo, n)
        for t in range(QT):
            par, j = divmod(c0 + t, half)
            if part == 0:
                qa[par, j, rows, :] = _tile(y, t) * (QK_SCALE * LOG2E)
                continue
            dst = ka if part == 1 else va
            dst[par, half + j, rows, :] = _tile(y, t)
            if j > 0:
                moved = pltpu.roll(_tile(y, t), 1, 1)
                if part == 2:
                    first = lax.broadcasted_iota(jnp.int32, moved.shape, 1) == 0
                    moved = jnp.where(first, va[0, half, rows, :], moved)
                dst[par, j, rows, :] = moved

    def a_qkv_steps(c0, n=ROWS):
        return [partial(a_qkv, c0, part, lo, n) for part in range(3) for lo in range(0, D, n)]

    def a_attend_steps(par, j, hg):
        logit, prob, res = {}, {}, {}

        def rows(sub, d):
            return pl.ds(d * H + hg * 16 + sub * 8, 8)

        def score(sub, d):
            qd = paced(qa[par, j, rows(sub, d), :], d)
            for w in range(WIN):
                term = qd * ka[par, half + j - w, rows(sub, d), :]
                logit[sub, w] = term if d == 0 else logit[sub, w] + term

        def soften(sub):
            lg = [logit[sub, w] if w <= j else jnp.where(lane == 0, MASKED * LOG2E, logit[sub, w])
                  for w in range(WIN)]
            top = reduce(jnp.maximum, lg)
            e = [jnp.exp2(x - top) for x in lg]
            inv = 1.0 / reduce(jnp.add, e)
            prob[sub] = [x * inv for x in e]

        def mix(sub, d):
            prob[sub] = [paced(prob[sub][0], d)] + prob[sub][1:]
            res[sub, d] = reduce(jnp.add, [prob[sub][w] * va[par, half + j - w, rows(sub, d), :]
                                           for w in range(WIN)])
            if sub == 1:
                pair = jnp.concatenate([res[0, d], res[1, d]], axis=0)
                ot[par * half + j, pl.ds(d * H + hg * 16, 16), :] = pair.astype(BF16)

        steps = []
        for sub in range(2):
            steps += [partial(score, sub, d) for d in range(DH)] + [partial(soften, sub)]
        return steps + [partial(mix, sub, d) for d in range(DH) for sub in range(2)]

    def a_attend(par):
        return [step for j in range(half) for hg in range(H // 16)
                for step in a_attend_steps(par, j, hg)]

    def b_keys(h, c):
        shift = (LANES - (h % GROUP) * DH) % LANES
        return pltpu.roll(kf[h // GROUP, c], shift, 1)

    def spread_keys(h, c):
        keys = b_keys(h, c)
        kq[c][...] = keys.astype(BF16)
        keys = keys[MXU_KEYS:, :]
        for d in range(DH):
            copies = jnp.broadcast_to(keys[:, d:d + 1], keys.shape)
            kl[c][0, d] = copies
            yield copies

    def b_qkv(c0, part, lo, n):
        y = project(wb_t, part * D + lo, n, xn, c0)
        rows = pl.ds(lo, n)
        if part == 0:
            y = y * (QK_SCALE * LOG2E)
            qf[c0 // QT, pl.ds(lo // DH, n // DH)] = y.reshape(n // DH, DH, QW)
        for t in range(QT):
            if part == 1:
                for g in range(n // LANES):
                    kf[lo // LANES + g, c0 + t] = _tile(y, t)[g * LANES:(g + 1) * LANES, :].T
            else:
                (qb if part == 0 else vb)[c0 + t, rows, :] = _tile(y, t).astype(BF16)

    def b_qkv_steps(c0, n=ROWS):
        return [partial(b_qkv, c0, part, lo, n) for part in (1, 0, 2) for lo in range(0, D, n)]

    def b_query(h, c0):
        r0 = pl.multiple_of(h * DH, DH)
        return _lanes([qb[c0 + t, pl.ds(r0, DH), :] for t in range(QT)])

    def normalise(num, den, bad):
        total = jnp.sum(den, axis=0, keepdims=True)
        ok = (total >= SUM_LO) & (total <= SUM_HI) & (jnp.abs(num) <= ACC_HI)
        return (num * (1.0 / total)).astype(BF16), jnp.where(ok, bad, 1.0)

    def head_rows(h):
        return pl.ds(pl.multiple_of(h * DH, DH), DH)

    def b_head(h, n, bad, pending, fetched, zero, sums):
        before, after = jnp.maximum(h - HEADS_PER_STEP, 0), jnp.minimum(h + 1, H - 1)
        acc, den = {}, [None] * NT

        def weigh(blk, c, p):
            part = jnp.dot(vb[c, head_rows(h), :], p, preferred_element_type=F32)
            if c == 0 and n > 0:
                never = jnp.tile(pace["never"].astype(jnp.int32), (DH // 8, QT)) > 0
                part = jnp.where(never, sums[n - 1][0][blk], part)
            acc[blk] = part if c == 0 else acc[blk] + part

        def vpu_weights(blk, c, offset, out):
            for r in range(VPU_KEYS // 8):
                s = [None] * QT
                for d in range(DH):
                    kd = kl[c][offset, d, r * 8:(r + 1) * 8, :]
                    for t in range(QT):
                        qd = jnp.broadcast_to(qf[blk, h + offset, d:d + 1, chunk(t)], (8, LANES))
                        s[t] = kd * qd if d == 0 else s[t] + kd * qd
                    if d == DH - 1:
                        out.append([jnp.exp2(st) for st in s])
                    yield

        def add_up(blk, rows):
            for t in range(QT):
                i = blk * QT + t
                for row in rows:
                    den[i] = row[t] if den[i] is None else den[i] + row[t]

        stages = DH * VPU_KEYS // 8
        queries = [b_query(h, blk * QT) for blk in range(NB)]
        for c in range(NT):
            if c + KEYS_AHEAD < NT:
                prefetch = spread_keys(h, c + KEYS_AHEAD)
            else:
                prefetch = spread_keys(after, c + KEYS_AHEAD - NT)
            shared = n > 0 or c > 0
            keys = MXU_KEYS if shared else LANES
            for blk in range(NB):
                s = jnp.dot(kq[c][:keys, :DH], queries[blk], preferred_element_type=F32)
                rows, extra, done = [], [], 0
                side = vpu_weights(blk, c, zero[blk], extra)
                for r in range(keys // 8):
                    rows.append([jnp.exp2(_tile(s, t)[r * 8:(r + 1) * 8, :]) for t in range(QT)])
                    if r % 2 == 1:
                        add_up(blk, rows[-2:])
                    upto = (r + 1) * stages // (keys // 8) if shared else 0
                    for _ in range(done, upto):
                        next(side)
                    done = upto
                    if r % 3 == 2 and r < 12:
                        fetched.append(next(prefetch))
                add_up(blk, extra)
                while len(fetched) > (TIE_LAG if shared else 0):
                    old = fetched.pop(0)
                    if shared and len(fetched) == TIE_LAG:
                        extra[-1][0] = jnp.where(pace["never"], old[8:], extra[-1][0])
                p = jnp.concatenate([_lanes(row) for row in rows + extra], axis=0)
                pending.append(partial(weigh, blk, c, p.astype(BF16)))
                if len(pending) > PV_LAG:
                    pending.pop(0)()
                if blk == 1:
                    done_tile, bad = normalise(nums[n, c], dens[n, c], bad)
                if blk == NB - 1:
                    ot[c, head_rows(before), :] = done_tile
        return bad, acc, den

    def b_fast(i, bad):
        zero = [i // (H + 1 + 2 * blk) for blk in range(NB)]
        pending, fetched, sums = [], [], []
        for n in range(HEADS_PER_STEP):
            bad, acc, den = b_head(i * HEADS_PER_STEP + n, n, bad, pending, fetched, zero, sums)
            sums.append((acc, den))
        for last in pending:
            last()
        for n, (acc, den) in enumerate(sums):
            for c in range(NT):
                nums[n, c], dens[n, c] = _tile(acc[c // QT], c % QT), den[c]
        return bad

    def first_keys(c):
        for _ in spread_keys(0, c):
            pass

    def b_attend():
        nums[...] = jnp.zeros(nums.shape, F32)
        dens[...] = jnp.ones(dens.shape, F32)
        bad = lax.fori_loop(0, H // HEADS_PER_STEP, b_fast, jnp.zeros((DH, LANES), F32))
        for n in range(HEADS_PER_STEP):
            rows = pl.ds((H - HEADS_PER_STEP + n) * DH, DH)
            for c in range(NT):
                ot[c, rows, :], bad = normalise(nums[n, c], dens[n, c], bad)

        @pl.when(jnp.max(bad) > 0.0)
        def _():
            lax.fori_loop(0, (NT // QT) * H, b_safe, 0)

    def b_safe(i, carry):
        c0 = (i // H) * QT
        h = i % H
        r0 = pl.multiple_of(h * DH, DH)
        q = b_query(h, c0)

        def step(c, state):
            top, den, acc = state
            keys = b_keys(h, c)[:, :DH].astype(BF16)
            s = jnp.dot(keys, q, preferred_element_type=F32)
            new_top = jnp.maximum(top, jnp.max(s, axis=0, keepdims=True))
            keep = jnp.exp2(top - new_top)
            p = jnp.exp2(s - new_top)
            den = den * keep + jnp.sum(p, axis=0, keepdims=True)
            acc = acc * keep + jnp.dot(vb[c, pl.ds(r0, DH), :], p.astype(BF16),
                                       preferred_element_type=F32)
            return new_top, den, acc

        init = (jnp.full((1, QW), -jnp.inf, F32), jnp.zeros((1, QW), F32),
                jnp.zeros((DH, QW), F32))
        _, den, acc = lax.fori_loop(0, NT, step, init)
        out = acc / den
        for t in range(QT):
            ot[c0 + t, pl.ds(r0, DH), :] = _tile(out, t).astype(BF16)
        return carry

    for pair in range(2):
        if pair == 0:
            _weave(norms(0))
            first, second = a_qkv_steps(0), a_qkv_steps(QT)
            n = len(first) // 3
            _weave(first[:n], norms(QT))
            wa_loads[1].wait()
            wa_loads[2].wait()
            _weave(second[:n], [partial(prepare_wqkv_a, 1, kt) for kt in range(KT)])
            _weave(first[n:2 * n] + second[n:2 * n],
                   [partial(prepare_wqkv_a, 2, kt) for kt in range(KT)])
            _weave(first[2 * n:] + second[2 * n:], norms(2 * QT) + norms(3 * QT))
        else:
            _weave(out_steps(wob_t, 0))
            _weave(out_steps(wob_t, QT) + out_steps(wob_t, 2 * QT) + out_steps(wob_t, 3 * QT),
                   norms(0) + norms(QT))
            _weave(a_qkv_steps(0) + a_qkv_steps(QT), norms(2 * QT) + norms(3 * QT))
        extra = []
        if pair == 0:
            for cp in late_loads:
                cp.wait()
            extra = late_weights()
        _weave(a_qkv_steps(2 * QT) + a_qkv_steps(3 * QT), a_attend(0), extra)
        _weave(out_steps(woa_t, 0) + out_steps(woa_t, QT) + norms(0) + norms(QT)
               + b_qkv_steps(0) + b_qkv_steps(QT), a_attend(1))
        _weave(out_steps(woa_t, 2 * QT))
        _weave(out_steps(woa_t, 3 * QT), norms(2 * QT))
        _weave(b_qkv_steps(2 * QT), norms(3 * QT),
               [partial(first_keys, c) for c in range(KEYS_AHEAD)])
        _weave(b_qkv_steps(3 * QT))
        b_attend()

    stores = [pltpu.make_async_copy(x_io.at[i], out_hbm.at[:, chunk(i)], sems.at[i])
              for i in range(KT)]

    def store_tile(ft, j):
        even = pltpu.bitcast(xt[j, chunk(ft), :].astype(BF16).astype(F32), U32)
        odd = pltpu.bitcast(xt[half + j, chunk(ft), :].astype(BF16).astype(F32), U32)
        stage_x[ft, pl.ds(j, LANES, stride=half), :] = ((even >> 16) | odd).T

    for ft in range(KT + 1):
        last = [partial(out_project, wob_t, c0, ft * LANES, LANES)
                for c0 in range(0, NT, QT)] if ft < KT else []
        _weave(last, [partial(store_tile, ft - 1, j) for j in range(half)] if ft > 0 else [])
        if ft > 0:
            x_io[ft - 1] = pltpu.bitcast(stage_x[ft - 1], BF16)
            stores[ft - 1].start()
    for cp in stores:
        cp.wait()


@jax.jit
def pallas_interleave_layers__sliding_local_dilated__softmax_full_mha__prompt_kernel(
    A_x: jax.Array,
    A_wqkv: jax.Array,
    A_wo: jax.Array,
    B_x: jax.Array,
    B_wqkv: jax.Array,
    B_wo: jax.Array,
):
    del B_x
    assert A_x.shape == (1, S, D) and A_x.dtype == BF16
    hbm = pl.BlockSpec(memory_space=pl.ANY)
    out = pl.pallas_call(
        _kernel,
        out_shape=jax.ShapeDtypeStruct((S, D), BF16),
        in_specs=[hbm] * 5,
        out_specs=hbm,
        scratch_shapes=[
            pltpu.VMEM((KT, S, LANES), BF16),
            pltpu.VMEM((3, D, D), BF16),
            pltpu.VMEM((D, D), BF16),
            pltpu.VMEM((D, 3 * D), BF16),
            pltpu.VMEM((D, D), BF16),
            pltpu.VMEM((KT, 3 * D, LANES), F32),
            pltpu.VMEM((KT, S // 2, LANES), U32),
            pltpu.VMEM((KT, 3 * D, LANES), BF16),
            pltpu.VMEM((KT, D, LANES), BF16),
            pltpu.VMEM((KT, 3 * D, LANES), BF16),
            pltpu.VMEM((KT, D, LANES), BF16),
            pltpu.VMEM((NT, D, LANES), F32),
            pltpu.VMEM((NT, D, LANES), BF16),
            pltpu.VMEM((2, NT // 2, D, LANES), F32),
            pltpu.VMEM((2, NT, D, LANES), F32),
            pltpu.VMEM((2, NT, D, LANES), F32),
            pltpu.VMEM((NT, D, LANES), BF16),
            pltpu.VMEM((NT, D, LANES), BF16),
            pltpu.VMEM((NT // QT, H, DH, QW), F32),
            pltpu.VMEM((KT, NT, LANES, LANES), F32),
            pltpu.VMEM((NT, D, LANES), BF16),
            pltpu.VMEM((HEADS_PER_STEP, NT, DH, LANES), F32),
            pltpu.VMEM((HEADS_PER_STEP, NT, 8, LANES), F32),
            pltpu.SemaphoreType.DMA((KT + 6,)),
            *[pltpu.VMEM((LANES, LANES), BF16)] * NT,
            *[pltpu.VMEM((1, DH, VPU_KEYS, LANES), F32)] * NT,
        ],
        compiler_params=pltpu.CompilerParams(vmem_limit_bytes=100 * 1024 * 1024),
    )(A_x.reshape(S, D), A_wqkv, A_wo, B_wqkv, B_wo)
    return out.reshape(1, S, D)
```
